```python
import os as _os
_os.environ.setdefault('JAX_PLATFORMS', 'cpu')
import jax
import jax.numpy as jnp

def _softmax(x, axis=-1):
    return jax.nn.softmax(x, axis=axis)

def _gelu(x):
    return jax.nn.gelu(x, approximate=True)

def _silu(x):
    return jax.nn.silu(x)

def _sigmoid(x):
    return jax.nn.sigmoid(x)

def _layernorm(x, axis=-1, eps=1e-05):
    m = jnp.mean(x, axis=axis, keepdims=True)
    v = jnp.var(x, axis=axis, keepdims=True)
    return (x - m) / jnp.sqrt(v + eps)

def _scatter_add(tgt, idx, src, axis=0):
    return tgt.at[idx].add(src)

def _segment_sum(src, seg, n):
    return jax.ops.segment_sum(src, seg, n)

class _Rng:

    def __init__(self, key):
        self._k = key

    def _next(self):
        self._k, sub = jax.random.split(self._k)
        return sub

    def normal(self, shape):
        return jax.random.normal(self._next(), shape, dtype=jnp.bfloat16)

    def randint(self, lo, hi, shape):
        return jax.random.randint(self._next(), shape, lo, hi, dtype=jnp.int32)

    def uniform(self, shape, lo=0.0, hi=1.0):
        return jax.random.uniform(self._next(), shape, jnp.bfloat16, lo, hi)

    def permutation(self, n):
        return jax.random.permutation(self._next(), n)
kernel_name = 'standalone__conformer_conv_module__speech'

def setup_inputs():
    _rng = _Rng(jax.random.key(int.from_bytes(__import__("os").urandom(4), "little")))
    _w = lambda a: (lambda t: t.astype(jnp.bfloat16) if jnp.issubdtype(t.dtype, jnp.floating) else t)(jnp.asarray(a))
    B, T, D, K = (2, 4000, 512, 15)
    return {'x': _w((lambda *s: _rng.normal(s) * 0.2)(B, T, D)), 'w_pw1': _w((lambda *s: _rng.normal(s) * 0.2)(D, 2 * D)), 'dw': _w((lambda *s: _rng.normal(s) * 0.05)(K, D)), 'w_pw2': _w((lambda *s: _rng.normal(s) * 0.05)(D, D))}

def reference(x, w_pw1, dw, w_pw2):
    B, T, D = x.shape
    K = dw.shape[0]
    h = x @ w_pw1
    a, b = (h[..., :D].copy(), h[..., D:].copy())
    h = a * _sigmoid(b)
    pad = K // 2
    hp = jnp.pad(h, ((0, 0), (pad, pad), (0, 0)))
    out = jnp.zeros_like(h)
    for i in range(K):
        out = out + hp[:, i:i + T, :] * dw[i][None, None, :]
    return _silu(out) @ w_pw2
```

```python
import functools
import jax
import jax.numpy as jnp
from jax import lax
import jax.experimental.pallas as pl
import jax.experimental.pallas.tpu as pltpu

TT = 800
OFFS = (1,2,3,4)
ORDER = 1

def _kernel(x_ref, w1_ref, dw_ref, w2_ref, o_ref, h_ref, p_ref, dwb_ref, acc_ref, *, n_tiles, tiles_per_batch, K, D):
    i = pl.program_id(0)
    NC = D // 128
    P = K // 2
    G = n_tiles * TT
    NV = TT // 8
    base = pl.multiple_of(i * TT, 8)

    @pl.when(i == 0)
    def _():
        z = jnp.zeros((8, 128), jnp.float32)
        for c in range(NC):
            h_ref[c, pl.ds(TT, 8), :] = z
            h_ref[c, pl.ds(TT + 8 + G, 8), :] = z
        dwf = dw_ref[...].astype(jnp.float32) * 0.25
        for k in range(K):
            for c in range(NC):
                dwb_ref[c, k] = jnp.broadcast_to(dwf[k:k + 1, c * 128:(c + 1) * 128], (8, 128))

    def f_pass(c, x):
        return jnp.dot(x, w1_ref[:, c * 128:(c + 1) * 128], preferred_element_type=jnp.float32)

    def g_pass(c, x, a):
        g = jnp.dot(x, w1_ref[:, D + c * 128:D + (c + 1) * 128], preferred_element_type=jnp.float32)
        h = a + a * jnp.tanh(0.5 * g)
        h_ref[c, pl.ds(base + (TT + 8), TT), :] = h
        hprev = h_ref[c, pl.ds(base + TT, 8), :]
        h3 = h.reshape(NV, 8, 128)
        hm = jnp.concatenate([hprev[None], h3[:-1]], axis=0)
        for oi, o in enumerate(OFFS):
            pv = h3 * dwb_ref[c, P + o][None] + hm * dwb_ref[c, o - 1][None]
            p_ref[oi, c, pl.ds(base + (TT + 8), TT), :] = pv.reshape(TT, 128)

    def conv(c):
        j = i - 1
        jb = j % tiles_per_batch
        first = jb == 0
        last = jb == tiles_per_batch - 1
        rows = lax.broadcasted_iota(jnp.int32, (8, 128), 0)
        def edge(r0, is_first):
            acc = None
            for k in range(K):
                hv = h_ref[c, pl.ds(base + (8 + k - P + r0), 8), :]
                if is_first and k < P:
                    hv = jnp.where(rows >= jnp.where(first, P - k, 0), hv, 0.0)
                if (not is_first) and k > P:
                    hv = jnp.where(rows < jnp.where(last, 8 - (k - P), 8), hv, 0.0)
                t = hv * dwb_ref[c, k]
                acc = t if acc is None else acc + t
            return acc
        y0 = edge(0, True)
        y1 = edge(TT - 8, False)
        nr = TT - 16
        acc = None
        for k in range(K):
            o = k - P
            if o in OFFS or (o + 8) in OFFS:
                continue
            hv = h_ref[c, pl.ds(base + (16 + o), nr), :].reshape(nr // 8, 8, 128)
            t = hv * dwb_ref[c, k][None]
            acc = t if acc is None else acc + t
        for oi, o in enumerate(OFFS):
            acc = acc + p_ref[oi, c, pl.ds(base + (16 + o), nr), :].reshape(nr // 8, 8, 128)
        y = jnp.concatenate([y0[None], acc, y1[None]], axis=0).reshape(TT, 128)
        return (y + y * jnp.tanh(y)).astype(jnp.bfloat16)

    def mm2(c):
        p = jnp.dot(conv(c), w2_ref[c * 128:(c + 1) * 128, :], preferred_element_type=jnp.float32)
        if c == 0:
            acc_ref[...] = p
        elif c < NC - 1:
            acc_ref[...] += p
        else:
            o_ref[...] = (acc_ref[...] + p).astype(o_ref.dtype)

    @pl.when(i == 0)
    def _():
        x = x_ref[...]
        for c in range(NC):
            g_pass(c, x, f_pass(c, x))

    @pl.when(jnp.logical_and(i > 0, i < n_tiles))
    def _():
        x = x_ref[...]
        if ORDER == 0:
            for c in range(NC):
                g_pass(c, x, f_pass(c, x))
                mm2(c)
        else:
            a = f_pass(0, x)
            for c in range(NC):
                g_pass(c, x, a)
                if c + 1 < NC:
                    a = f_pass(c + 1, x)
                mm2(c)

    @pl.when(i == n_tiles)
    def _():
        for c in range(NC):
            mm2(c)


@jax.jit
def pallas_standalone__conformer_conv_module__speech_kernel(x, w_pw1, dw, w_pw2):
    B, T, D = x.shape
    K = dw.shape[0]
    x2 = x.reshape(B * T, D)
    n_tiles = B * T // TT
    tpb = T // TT
    NC = D // 128
    kern = functools.partial(_kernel, n_tiles=n_tiles, tiles_per_batch=tpb, K=K, D=D)
    out = pl.pallas_call(
        kern,
        grid=(n_tiles + 1,),
        in_specs=[
            pl.BlockSpec((TT, D), lambda i: (jnp.minimum(i, n_tiles - 1), 0)),
            pl.BlockSpec((D, 2 * D), lambda i: (0, 0)),
            pl.BlockSpec((K, D), lambda i: (0, 0)),
            pl.BlockSpec((D, D), lambda i: (0, 0)),
        ],
        out_specs=pl.BlockSpec((TT, D), lambda i: (jnp.maximum(i - 1, 0), 0)),
        out_shape=jax.ShapeDtypeStruct((B * T, D), x.dtype),
        scratch_shapes=[
            pltpu.VMEM((NC, B * T + TT + 16, 128), jnp.float32),
            pltpu.VMEM((len(OFFS), NC, B * T + TT + 16, 128), jnp.float32),
            pltpu.VMEM((NC, K, 8, 128), jnp.float32),
            pltpu.VMEM((TT, D), jnp.float32),
        ],
        compiler_params=pltpu.CompilerParams(
            dimension_semantics=("arbitrary",),
            vmem_limit_bytes=110 * 1024 * 1024,
        ),
    )(x2, w_pw1, dw, w_pw2)
    return out.reshape(B, T, D)
```

```python
import functools
import jax
import jax.numpy as jnp
from jax import lax
import jax.experimental.pallas as pl
import jax.experimental.pallas.tpu as pltpu

L = 960
LA = 480
NT = 5
OFFS = (1, 2, 3)
EPI = (480, 240, 112, 64, 32, 32)
OCH = 2
NOCHK = True
PROF = False


def _tree(terms):
    while len(terms) > 1:
        nt = [terms[j] + terms[j + 1] for j in range(0, len(terms) - 1, 2)]
        if len(terms) % 2:
            nt.append(terms[-1])
        terms = nt
    return terms[0]


def _split16(n, parts):
    g = n // 16
    q, r = divmod(g, parts)
    return [16 * (q + (1 if j < r else 0)) for j in range(parts) if q + (1 if j < r else 0) > 0]


def _kernel(x_hbm, w1_hbm, dw_hbm, w2_hbm, o_hbm,
            xb, w1b, w2b, dwb_in, ob, h_ref, p_ref, dwb_ref, acc_ref, w1u, w2u, sems,
            *, G, T, K, D, TT):
    NC = D // 128
    P = K // 2
    f32 = jnp.float32
    bf16 = jnp.bfloat16
    u32 = jnp.uint32
    H0 = 32

    S_W2, S_G1, S_G2, S_G3, S_G4, S_O, S_X = 0, 1, 2, 3, 4, 5, 6

    def wait(name, cps):
        if PROF:
            with jax.named_scope(name):
                for cp in cps:
                    cp.wait()
        else:
            for cp in cps:
                cp.wait()

    def w1_cp(r0, nr, c0, nc, s):
        sl = (pl.ds(r0, nr), pl.ds(c0, nc))
        return pltpu.make_async_copy(w1_hbm.at[sl], w1b.at[sl], sems.at[s])

    def x_cp2(r0, nr, c0, nc, s):
        sl = (pl.ds(r0, nr), pl.ds(c0, nc))
        return pltpu.make_async_copy(x_hbm.at[sl], xb.at[sl], sems.at[s])

    def x_cp(r0, nr, s):
        return pltpu.make_async_copy(x_hbm.at[pl.ds(r0, nr)], xb.at[pl.ds(r0, nr)], sems.at[s])

    def o_cp(r0, nr):
        return pltpu.make_async_copy(ob.at[pl.ds(r0, nr)], o_hbm.at[pl.ds(r0, nr)], sems.at[S_O])

    w2_cp = pltpu.make_async_copy(w2_hbm, w2b, sems.at[S_W2])
    g1 = [w1_cp(0, 128, 0, D, S_G1), x_cp2(0, LA, 0, 128, S_G1)]
    g2 = [x_cp2(LA, L - LA, 0, 128, S_G2), w1_cp(0, 128, D, D, S_G2)]
    g3 = [pltpu.make_async_copy(dw_hbm, dwb_in, sems.at[S_G3]),
          x_cp2(0, L, 128, 128, S_G3), w1_cp(128, 128, 0, 2 * D, S_G3)]
    g4 = [x_cp2(0, L, 256, 256, S_G4), w1_cp(256, 256, 0, 2 * D, S_G4)]

    for cp in g1 + g2 + g3 + g4:
        cp.start()
    w2_cp.start()
    for t in range(NT):
        x_cp(L + t * TT, TT, S_X + t).start()

    z = jnp.zeros((8, 128), f32)
    for c in range(NC):
        h_ref[c, pl.ds(H0 - 8, 8), :] = z
        h_ref[c, pl.ds(H0 + G, 8), :] = z

    def glu_store(c, a, g, r0, nr):
        h = a + a * jnp.tanh(0.5 * g)
        h_ref[c, pl.ds(r0 + H0, nr), :] = h
        hprev = h_ref[c, pl.ds(r0 + (H0 - 8), 8), :]
        h3 = h.reshape(nr // 8, 8, 128)
        hm = jnp.concatenate([hprev[None], h3[:-1]], axis=0)
        for oi, o in enumerate(OFFS):
            pv = h3 * dwb_ref[c, P + o][None] + hm * dwb_ref[c, o - 1][None]
            p_ref[oi, c, pl.ds(r0 + H0, nr), :] = pv.reshape(nr, 128)

    def f_pass(c, x):
        return jnp.dot(x, pltpu.bitcast(w1u[c], bf16), preferred_element_type=f32)

    def g_pass(c, x, a, r0, nr):
        g = jnp.dot(x, pltpu.bitcast(w1u[NC + c], bf16), preferred_element_type=f32)
        glu_store(c, a, g, r0, nr)

    rows = lax.broadcasted_iota(jnp.int32, (8, 128), 0)

    def conv_direct(c, r0, lo_pred=None, hi_pred=None):
        terms = []
        for k in range(K):
            hv = h_ref[c, pl.ds(r0 + (H0 + k - P), 8), :]
            if lo_pred is not None and k < P:
                hv = jnp.where(rows >= jnp.where(lo_pred, P - k, 0), hv, 0.0)
            if hi_pred is not None and k > P:
                hv = jnp.where(rows < jnp.where(hi_pred, 8 - (k - P), 8), hv, 0.0)
            terms.append(hv * dwb_ref[c, k])
        return _tree(terms)[None]

    def conv_paired(c, r0, nr):
        terms = []
        for k in range(K):
            o = k - P
            if o in OFFS or (o + 8) in OFFS:
                continue
            hv = h_ref[c, pl.ds(r0 + (H0 + o), nr), :].reshape(nr // 8, 8, 128)
            terms.append(hv * dwb_ref[c, k][None])
        for oi, o in enumerate(OFFS):
            terms.append(p_ref[oi, c, pl.ds(r0 + (H0 + o), nr), :].reshape(nr // 8, 8, 128))
        return _tree(terms)

    def conv(c, base, s0, nr, special):
        parts = []
        r = s0
        for sr in sorted(special):
            if s0 <= sr < s0 + nr:
                if sr > r:
                    parts.append(conv_paired(c, base + r, sr - r))
                parts.append(conv_direct(c, base + sr, **special[sr]))
                r = sr + 8
        if r < s0 + nr:
            parts.append(conv_paired(c, base + r, s0 + nr - r))
        y = jnp.concatenate(parts, axis=0) if len(parts) > 1 else parts[0]
        return y.reshape(nr, 128)

    def mm2(c, base, s0, nr, special, a0, och, first=False):
        y = conv(c, base, s0, nr, special)
        s = (y + y * jnp.tanh(y)).astype(bf16)
        if first:
            w = w2b[c * 128:(c + 1) * 128, :]
            w2u[c] = pltpu.bitcast(w, u32)
        else:
            w = pltpu.bitcast(w2u[c], bf16)
        p = jnp.dot(s, w, preferred_element_type=f32)
        if c == 0:
            acc_ref[pl.ds(a0, nr), :] = p
        elif c < NC - 1:
            acc_ref[pl.ds(a0, nr), :] += p
        else:
            q0 = 0
            for q in _split16(nr, och):
                ob[pl.ds(base + (s0 + q0), q), :] = (
                    acc_ref[pl.ds(a0 + q0, q), :] + p[q0:q0 + q]).astype(ob.dtype)
                o_cp(base + (s0 + q0), q).start()
                q0 += q

    def pk(k, half, r0, nr, pack):
        w = w1b[k * 128:(k + 1) * 128, half * D:(half + 1) * D]
        if pack:
            wu = pltpu.bitcast(w, u32)
            for c in range(NC):
                w1u[half * NC + c, k * 64:(k + 1) * 64, :] = wu[:, c * 128:(c + 1) * 128]
        p = jnp.dot(xb[pl.ds(r0, nr), k * 128:(k + 1) * 128], w, preferred_element_type=f32)
        if k == 0:
            acc_ref[pl.ds(half * L + r0, nr), :] = p
        else:
            acc_ref[pl.ds(half * L + r0, nr), :] += p

    wait("wait_g1", g1)
    pk(0, 0, 0, LA, False)
    wait("wait_g2", g2)
    pk(0, 0, LA, L - LA, True)
    pk(0, 1, 0, L, True)
    wait("wait_g3", g3)
    pk(1, 0, 0, L, True)
    dwf = dwb_in[...].astype(f32) * 0.25
    for k in range(K):
        for c in range(NC):
            dwb_ref[c, k] = jnp.broadcast_to(dwf[k:k + 1, c * 128:(c + 1) * 128], (8, 128))
    pk(1, 1, 0, L, True)
    wait("wait_g4", g4)
    x23 = xb[pl.ds(0, L), 256:512]
    for c in range(NC):
        wa = w1b[256:512, c * 128:(c + 1) * 128]
        wb = w1b[256:512, D + c * 128:D + (c + 1) * 128]
        w1u[c, 128:256, :] = pltpu.bitcast(wa, u32)
        w1u[NC + c, 128:256, :] = pltpu.bitcast(wb, u32)
        q = jnp.dot(x23, jnp.concatenate([wa, wb], axis=1), preferred_element_type=f32)
        a = acc_ref[pl.ds(0, L), c * 128:(c + 1) * 128] + q[:, :128]
        g = acc_ref[pl.ds(L, L), c * 128:(c + 1) * 128] + q[:, 128:]
        glu_store(c, a, g, 0, L)
    wait("wait_w2", [w2_cp])

    bt, boff = divmod(T, TT)
    assert G == 2 * T and boff % 8 == 0 and 8 <= boff <= TT - 8 and bt < NT
    RA = L - 16
    RB = TT - RA

    def body(i, carry):
        base = pl.multiple_of(i * TT, 32)
        wait("wait_x", [x_cp(L + base, TT, S_X + i)])
        at_b = i == bt
        special = {boff - 8: dict(hi_pred=at_b), boff: dict(lo_pred=at_b)}
        x = xb[pl.ds(base + L, TT), :]
        a = f_pass(0, x)
        mm2(0, base, 0, RA, special, 0, OCH, first=True)
        for c in range(NC):
            g_pass(c, x, a, base + L, TT)
            if c + 1 < NC:
                a = f_pass(c + 1, x)
                mm2(c + 1, base, 0, RA, special, 0, OCH, first=True)
            mm2(c, base, RA, RB, special, RA, OCH)
        return carry

    lax.fori_loop(0, NT, body, 0)

    r0 = NT * TT
    special = {G - 8: {}}
    for e, nr in enumerate(EPI):
        for c in range(NC):
            mm2(c, 0, r0, nr, special, r0 - NT * TT, 1)
        r0 += nr

    wait("wait_out", [pltpu.make_async_copy(ob, o_hbm, sems.at[S_O])])


@jax.jit
def pallas_standalone__conformer_conv_module__speech_kernel(x, w_pw1, dw, w_pw2):
    B, T, D = x.shape
    K = dw.shape[0]
    G = B * T
    x2 = x.reshape(G, D)
    NC = D // 128
    TT = (G - L) // NT
    assert L + NT * TT == G and TT % 32 == 0 and sum(EPI) == L
    kern = functools.partial(_kernel, G=G, T=T, K=K, D=D, TT=TT)
    out = pl.pallas_call(
        kern,
        in_specs=[pl.BlockSpec(memory_space=pl.ANY)] * 4,
        out_specs=pl.BlockSpec(memory_space=pl.ANY),
        out_shape=jax.ShapeDtypeStruct((G, D), x.dtype),
        scratch_shapes=[
            pltpu.VMEM((G, D), jnp.bfloat16),
            pltpu.VMEM((D, 2 * D), jnp.bfloat16),
            pltpu.VMEM((D, D), jnp.bfloat16),
            pltpu.VMEM((K, D), jnp.bfloat16),
            pltpu.VMEM((G, D), jnp.bfloat16),
            pltpu.VMEM((NC, G + 64, 128), jnp.float32),
            pltpu.VMEM((len(OFFS), NC, G + 64, 128), jnp.float32),
            pltpu.VMEM((NC, K, 8, 128), jnp.float32),
            pltpu.VMEM((max(TT, 2 * L), D), jnp.float32),
            pltpu.VMEM((2 * NC, D // 2, 128), jnp.uint32),
            pltpu.VMEM((NC, 64, D), jnp.uint32),
            pltpu.SemaphoreType.DMA((6 + NT,)),
        ],
        compiler_params=pltpu.CompilerParams(
            vmem_limit_bytes=120 * 1024 * 1024,
            disable_bounds_checks=NOCHK,
            disable_semaphore_checks=NOCHK,
        ),
    )(x2, w_pw1, dw, w_pw2)
    return out.reshape(B, T, D)
```

```python
import functools

import jax
import jax.numpy as jnp
from jax import lax
import jax.experimental.pallas as pl
import jax.experimental.pallas.tpu as pltpu

_LAG = 960
_L0 = 128
_L1 = 688
_NT = 5
_OFFS = (1, 2, 3, 4)
_EPI = (448, 256, 128, 64, 32, 32)
_H0 = 32


def _tree_sum(terms):
    while len(terms) > 1:
        nxt = [terms[j] + terms[j + 1] for j in range(0, len(terms) - 1, 2)]
        if len(terms) % 2:
            nxt.append(terms[-1])
        terms = nxt
    return terms[0]


def _kernel(x_hbm, w1_hbm, dw_hbm, w2_hbm, o_hbm,
            xb, w1b, w2b, dw_in, ob, h_ref, p_ref, dwb_ref, acc_ref, w1u, w2u, sems,
            *, G, T, K, D, TT):
    L, H0 = _LAG, _H0
    NC = D // 128
    P = K // 2
    f32, bf16, u32 = jnp.float32, jnp.bfloat16, jnp.uint32
    S_G0, S_G1, S_G2, S_G3, S_G4, S_W2, S_OUT, S_X = range(8)

    def w1_cp(r0, nr, c0, nc, s):
        sl = (pl.ds(r0, nr), pl.ds(c0, nc))
        return pltpu.make_async_copy(w1_hbm.at[sl], w1b.at[sl], sems.at[s])

    def xcol_cp(r0, nr, c0, nc, s):
        sl = (pl.ds(r0, nr), pl.ds(c0, nc))
        return pltpu.make_async_copy(x_hbm.at[sl], xb.at[sl], sems.at[s])

    def x_cp(r0, nr, s):
        return pltpu.make_async_copy(x_hbm.at[pl.ds(r0, nr)], xb.at[pl.ds(r0, nr)], sems.at[s])

    def o_cp(r0, nr):
        return pltpu.make_async_copy(ob.at[pl.ds(r0, nr)], o_hbm.at[pl.ds(r0, nr)], sems.at[S_OUT])

    def wait_all(cps):
        for cp in cps:
            cp.wait()

    g0 = [w1_cp(0, 128, 0, D, S_G0), xcol_cp(0, _L0, 0, 128, S_G0)]
    g1 = [xcol_cp(_L0, _L1 - _L0, 0, 128, S_G1)]
    g2 = [xcol_cp(_L1, L - _L1, 0, 128, S_G2), w1_cp(0, 128, D, D, S_G2)]
    g3 = [pltpu.make_async_copy(dw_hbm, dw_in, sems.at[S_G3]),
          xcol_cp(0, L, 128, 128, S_G3), w1_cp(128, 128, 0, 2 * D, S_G3)]
    g4 = [xcol_cp(0, L, 256, 256, S_G4), w1_cp(256, 256, 0, 2 * D, S_G4)]
    w2_cp = pltpu.make_async_copy(w2_hbm, w2b, sems.at[S_W2])

    for cp in g0 + g1 + g2 + g3 + g4 + [w2_cp]:
        cp.start()
    for t in range(_NT):
        x_cp(L + t * TT, TT, S_X + t).start()

    zero = jnp.zeros((8, 128), f32)
    for c in range(NC):
        h_ref[c, pl.ds(H0 - 8, 8), :] = zero
        h_ref[c, pl.ds(H0 + G, 8), :] = zero

    def glu_store(c, a, g, r0, nr):
        h = a + a * jnp.tanh(0.5 * g)
        h_ref[c, pl.ds(r0 + H0, nr), :] = h
        hprev = h_ref[c, pl.ds(r0 + (H0 - 8), 8), :]
        h3 = h.reshape(nr // 8, 8, 128)
        hm = jnp.concatenate([hprev[None], h3[:-1]], axis=0)
        for oi, o in enumerate(_OFFS):
            pv = h3 * dwb_ref[c, P + o][None] + hm * dwb_ref[c, o - 1][None]
            p_ref[oi, c, pl.ds(r0 + H0, nr), :] = pv.reshape(nr, 128)

    def a_pass(c, x):
        return jnp.dot(x, pltpu.bitcast(w1u[c], bf16), preferred_element_type=f32)

    def g_pass(c, x, a, r0, nr):
        g = jnp.dot(x, pltpu.bitcast(w1u[NC + c], bf16), preferred_element_type=f32)
        glu_store(c, a, g, r0, nr)

    rows = lax.broadcasted_iota(jnp.int32, (8, 128), 0)

    def conv_direct(c, r0, lo_pred=None, hi_pred=None):
        terms = []
        for k in range(K):
            hv = h_ref[c, pl.ds(r0 + (H0 + k - P), 8), :]
            if lo_pred is not None and k < P:
                hv = jnp.where(rows >= jnp.where(lo_pred, P - k, 0), hv, 0.0)
            if hi_pred is not None and k > P:
                hv = jnp.where(rows < jnp.where(hi_pred, 8 - (k - P), 8), hv, 0.0)
            terms.append(hv * dwb_ref[c, k])
        return _tree_sum(terms)[None]

    def conv_paired(c, r0, nr):
        terms = []
        for k in range(K):
            o = k - P
            if o in _OFFS or (o + 8) in _OFFS:
                continue
            hv = h_ref[c, pl.ds(r0 + (H0 + o), nr), :].reshape(nr // 8, 8, 128)
            terms.append(hv * dwb_ref[c, k][None])
        for oi, o in enumerate(_OFFS):
            terms.append(p_ref[oi, c, pl.ds(r0 + (H0 + o), nr), :].reshape(nr // 8, 8, 128))
        return _tree_sum(terms)

    def conv(c, base, s0, nr, direct):
        parts = []
        r = s0
        for sr in sorted(direct):
            if s0 <= sr < s0 + nr:
                if sr > r:
                    parts.append(conv_paired(c, base + r, sr - r))
                parts.append(conv_direct(c, base + sr, **direct[sr]))
                r = sr + 8
        if r < s0 + nr:
            parts.append(conv_paired(c, base + r, s0 + nr - r))
        y = jnp.concatenate(parts, axis=0) if len(parts) > 1 else parts[0]
        return y.reshape(nr, 128)

    def out_pass(c, base, s0, nr, direct, a0, pack_w=False):
        y = conv(c, base, s0, nr, direct)
        s = (y + y * jnp.tanh(y)).astype(bf16)
        if pack_w:
            w = w2b[c * 128:(c + 1) * 128, :]
            w2u[c] = pltpu.bitcast(w, u32)
        else:
            w = pltpu.bitcast(w2u[c], bf16)
        p = jnp.dot(s, w, preferred_element_type=f32)
        if c == 0:
            acc_ref[pl.ds(a0, nr), :] = p
        elif c < NC - 1:
            acc_ref[pl.ds(a0, nr), :] += p
        else:
            ob[pl.ds(base + s0, nr), :] = (acc_ref[pl.ds(a0, nr), :] + p).astype(ob.dtype)
            o_cp(base + s0, nr).start()

    def k_pass(k, half, r0, nr, pack_w):
        w = w1b[k * 128:(k + 1) * 128, half * D:(half + 1) * D]
        if pack_w:
            wu = pltpu.bitcast(w, u32)
            for c in range(NC):
                w1u[half * NC + c, k * 64:(k + 1) * 64, :] = wu[:, c * 128:(c + 1) * 128]
        p = jnp.dot(xb[pl.ds(r0, nr), k * 128:(k + 1) * 128], w, preferred_element_type=f32)
        if k == 0:
            acc_ref[pl.ds(half * L + r0, nr), :] = p
        else:
            acc_ref[pl.ds(half * L + r0, nr), :] += p

    wait_all(g0)
    k_pass(0, 0, 0, _L0, False)
    wait_all(g1)
    k_pass(0, 0, _L0, _L1 - _L0, False)
    wait_all(g2)
    k_pass(0, 0, _L1, L - _L1, True)
    k_pass(0, 1, 0, L, True)
    wait_all(g3)
    k_pass(1, 0, 0, L, True)
    dwf = dw_in[...].astype(f32) * 0.25
    for k in range(K):
        for c in range(NC):
            dwb_ref[c, k] = jnp.broadcast_to(dwf[k:k + 1, c * 128:(c + 1) * 128], (8, 128))
    k_pass(1, 1, 0, L, True)
    wait_all(g4)
    x23 = xb[pl.ds(0, L), 256:512]
    for c in range(NC):
        wa = w1b[256:512, c * 128:(c + 1) * 128]
        wg = w1b[256:512, D + c * 128:D + (c + 1) * 128]
        w1u[c, 128:256, :] = pltpu.bitcast(wa, u32)
        w1u[NC + c, 128:256, :] = pltpu.bitcast(wg, u32)
        q = jnp.dot(x23, jnp.concatenate([wa, wg], axis=1), preferred_element_type=f32)
        a = acc_ref[pl.ds(0, L), c * 128:(c + 1) * 128] + q[:, :128]
        g = acc_ref[pl.ds(L, L), c * 128:(c + 1) * 128] + q[:, 128:]
        glu_store(c, a, g, 0, L)
    w2_cp.wait()

    bt, boff = divmod(T, TT)
    RA = L - 16
    RB = TT - RA

    def body(i, carry):
        base = pl.multiple_of(i * TT, 32)
        x_cp(L + base, TT, S_X + i).wait()
        at_b = i == bt
        direct = {boff - 8: dict(hi_pred=at_b), boff: dict(lo_pred=at_b)}
        x = xb[pl.ds(base + L, TT), :]
        a = a_pass(0, x)
        out_pass(0, base, 0, RA, direct, 0, pack_w=True)
        for c in range(NC):
            g_pass(c, x, a, base + L, TT)
            if c + 1 < NC:
                a = a_pass(c + 1, x)
                out_pass(c + 1, base, 0, RA, direct, 0, pack_w=True)
            out_pass(c, base, RA, RB, direct, RA)
        return carry

    lax.fori_loop(0, _NT, body, 0)

    r0 = _NT * TT
    for nr in _EPI:
        for c in range(NC):
            out_pass(c, 0, r0, nr, {G - 8: {}}, r0 - _NT * TT)
        r0 += nr

    pltpu.make_async_copy(ob, o_hbm, sems.at[S_OUT]).wait()


@jax.jit
def pallas_standalone__conformer_conv_module__speech_kernel(
    x: jax.Array,
    w_pw1: jax.Array,
    dw: jax.Array,
    w_pw2: jax.Array,
):
    B, T, D = x.shape
    K = dw.shape[0]
    G = B * T
    NC = D // 128
    TT = (G - _LAG) // _NT
    boff = T % TT
    assert B == 2 and D == 512 and K == 15
    assert _LAG + _NT * TT == G and TT % 32 == 0 and sum(_EPI) == _LAG and _LAG - 16 < TT
    assert T < _NT * TT and boff % 8 == 0 and 8 <= boff <= TT - 8

    kernel = functools.partial(_kernel, G=G, T=T, K=K, D=D, TT=TT)
    out = pl.pallas_call(
        kernel,
        in_specs=[pl.BlockSpec(memory_space=pl.ANY)] * 4,
        out_specs=pl.BlockSpec(memory_space=pl.ANY),
        out_shape=jax.ShapeDtypeStruct((G, D), x.dtype),
        scratch_shapes=[
            pltpu.VMEM((G, D), jnp.bfloat16),
            pltpu.VMEM((D, 2 * D), jnp.bfloat16),
            pltpu.VMEM((D, D), jnp.bfloat16),
            pltpu.VMEM((K, D), jnp.bfloat16),
            pltpu.VMEM((G, D), jnp.bfloat16),
            pltpu.VMEM((NC, G + 2 * _H0, 128), jnp.float32),
            pltpu.VMEM((len(_OFFS), NC, G + 2 * _H0, 128), jnp.float32),
            pltpu.VMEM((NC, K, 8, 128), jnp.float32),
            pltpu.VMEM((max(TT, 2 * _LAG), D), jnp.float32),
            pltpu.VMEM((2 * NC, D // 2, 128), jnp.uint32),
            pltpu.VMEM((NC, 64, D), jnp.uint32),
            pltpu.SemaphoreType.DMA((7 + _NT,)),
        ],
        compiler_params=pltpu.CompilerParams(
            vmem_limit_bytes=120 * 1024 * 1024,
            disable_bounds_checks=True,
            disable_semaphore_checks=True,
        ),
    )(x.reshape(G, D), w_pw1, dw, w_pw2)
    return out.reshape(B, T, D)
```

```python
import functools

import jax
import jax.numpy as jnp
from jax import lax
import jax.experimental.pallas as pl
import jax.experimental.pallas.tpu as pltpu

_LAG = 960
_L0 = 128
_L1 = 688
_NT = 5
_OFFS = ((1, 2, 3), (1, 2, 3, 4), (1, 2, 3, 4), (1, 2, 3))
_PBASE = (0, 3, 7, 11, 14)
_EPI = (448, 256, 128, 64, 32, 32)
_H0 = 32


def _tree_sum(terms):
    while len(terms) > 1:
        nxt = [terms[j] + terms[j + 1] for j in range(0, len(terms) - 1, 2)]
        if len(terms) % 2:
            nxt.append(terms[-1])
        terms = nxt
    return terms[0]


def _kernel(x_hbm, w1_hbm, dw_hbm, w2_hbm, o_hbm,
            xb, w1b, w2b, dw_in, ob, h_ref, p_ref, dwb_ref, acc_ref, w1u, w2u, sems,
            *, G, T, K, D, TT):
    L, H0 = _LAG, _H0
    NC = D // 128
    P = K // 2
    f32, bf16, u32 = jnp.float32, jnp.bfloat16, jnp.uint32
    S_G0, S_G1, S_G2, S_G3, S_G4, S_W2, S_OUT, S_X = range(8)

    def w1_cp(r0, nr, c0, nc, s):
        sl = (pl.ds(r0, nr), pl.ds(c0, nc))
        return pltpu.make_async_copy(w1_hbm.at[sl], w1b.at[sl], sems.at[s])

    def xcol_cp(r0, nr, c0, nc, s):
        sl = (pl.ds(r0, nr), pl.ds(c0, nc))
        return pltpu.make_async_copy(x_hbm.at[sl], xb.at[sl], sems.at[s])

    def x_cp(r0, nr, s):
        return pltpu.make_async_copy(x_hbm.at[pl.ds(r0, nr)], xb.at[pl.ds(r0, nr)], sems.at[s])

    def o_cp(r0, nr):
        return pltpu.make_async_copy(ob.at[pl.ds(r0, nr)], o_hbm.at[pl.ds(r0, nr)], sems.at[S_OUT])

    def wait_all(cps):
        for cp in cps:
            cp.wait()

    g0 = [w1_cp(0, 128, 0, D, S_G0), xcol_cp(0, _L0, 0, 128, S_G0)]
    g1 = [xcol_cp(_L0, _L1 - _L0, 0, 128, S_G1)]
    g2 = [xcol_cp(_L1, L - _L1, 0, 128, S_G2), w1_cp(0, 128, D, D, S_G2)]
    g3 = [pltpu.make_async_copy(dw_hbm, dw_in, sems.at[S_G3]),
          xcol_cp(0, L, 128, 128, S_G3), w1_cp(128, 128, 0, 2 * D, S_G3)]
    g4 = [xcol_cp(0, L, 256, 256, S_G4), w1_cp(256, 256, 0, 2 * D, S_G4)]
    w2_cp = pltpu.make_async_copy(w2_hbm, w2b, sems.at[S_W2])

    for cp in g0 + g1 + g2 + g3 + g4 + [w2_cp]:
        cp.start()
    for t in range(_NT):
        x_cp(L + t * TT, TT, S_X + t).start()

    zero = jnp.zeros((8, 128), f32)
    for c in range(NC):
        h_ref[c, pl.ds(H0 - 8, 8), :] = zero
        h_ref[c, pl.ds(H0 + G, 8), :] = zero

    def glu_store(c, a, g, r0, nr):
        h = a + a * jnp.tanh(0.5 * g)
        h_ref[c, pl.ds(r0 + H0, nr), :] = h
        hprev = h_ref[c, pl.ds(r0 + (H0 - 8), 8), :]
        h3 = h.reshape(nr // 8, 8, 128)
        hm = jnp.concatenate([hprev[None], h3[:-1]], axis=0)
        for oi, o in enumerate(_OFFS[c]):
            pv = h3 * dwb_ref[c, P + o][None] + hm * dwb_ref[c, o - 1][None]
            p_ref[_PBASE[c] + oi, pl.ds(r0 + H0, nr), :] = pv.reshape(nr, 128)

    def a_pass(c, x):
        return jnp.dot(x, pltpu.bitcast(w1u[c], bf16), preferred_element_type=f32)

    def g_pass(c, x, a, r0, nr):
        g = jnp.dot(x, pltpu.bitcast(w1u[NC + c], bf16), preferred_element_type=f32)
        glu_store(c, a, g, r0, nr)

    rows = lax.broadcasted_iota(jnp.int32, (8, 128), 0)

    def conv_direct(c, r0, lo_pred=None, hi_pred=None):
        terms = []
        for k in range(K):
            hv = h_ref[c, pl.ds(r0 + (H0 + k - P), 8), :]
            if lo_pred is not None and k < P:
                hv = jnp.where(rows >= jnp.where(lo_pred, P - k, 0), hv, 0.0)
            if hi_pred is not None and k > P:
                hv = jnp.where(rows < jnp.where(hi_pred, 8 - (k - P), 8), hv, 0.0)
            terms.append(hv * dwb_ref[c, k])
        return _tree_sum(terms)[None]

    def conv_paired(c, r0, nr):
        terms = []
        for k in range(K):
            o = k - P
            if o in _OFFS[c] or (o + 8) in _OFFS[c]:
                continue
            hv = h_ref[c, pl.ds(r0 + (H0 + o), nr), :].reshape(nr // 8, 8, 128)
            terms.append(hv * dwb_ref[c, k][None])
        for oi, o in enumerate(_OFFS[c]):
            pv = p_ref[_PBASE[c] + oi, pl.ds(r0 + (H0 + o), nr), :]
            terms.append(pv.reshape(nr // 8, 8, 128))
        return _tree_sum(terms)

    def conv(c, base, s0, nr, direct):
        parts = []
        r = s0
        for sr in sorted(direct):
            if s0 <= sr < s0 + nr:
                if sr > r:
                    parts.append(conv_paired(c, base + r, sr - r))
                parts.append(conv_direct(c, base + sr, **direct[sr]))
                r = sr + 8
        if r < s0 + nr:
            parts.append(conv_paired(c, base + r, s0 + nr - r))
        y = jnp.concatenate(parts, axis=0) if len(parts) > 1 else parts[0]
        return y.reshape(nr, 128)

    def out_pass(c, base, s0, nr, direct, a0, pack_w=False):
        y = conv(c, base, s0, nr, direct)
        s = (y + y * jnp.tanh(y)).astype(bf16)
        if pack_w:
            w = w2b[c * 128:(c + 1) * 128, :]
            w2u[c] = pltpu.bitcast(w, u32)
        else:
            w = pltpu.bitcast(w2u[c], bf16)
        p = jnp.dot(s, w, preferred_element_type=f32)
        if c == 0:
            acc_ref[pl.ds(a0, nr), :] = p
        elif c < NC - 1:
            acc_ref[pl.ds(a0, nr), :] += p
        else:
            ob[pl.ds(base + s0, nr), :] = (acc_ref[pl.ds(a0, nr), :] + p).astype(ob.dtype)
            o_cp(base + s0, nr).start()

    def k_pass(k, half, r0, nr, pack_w):
        w = w1b[k * 128:(k + 1) * 128, half * D:(half + 1) * D]
        if pack_w:
            wu = pltpu.bitcast(w, u32)
            for c in range(NC):
                w1u[half * NC + c, k * 64:(k + 1) * 64, :] = wu[:, c * 128:(c + 1) * 128]
        p = jnp.dot(xb[pl.ds(r0, nr), k * 128:(k + 1) * 128], w, preferred_element_type=f32)
        if k == 0:
            acc_ref[pl.ds(half * L + r0, nr), :] = p
        else:
            acc_ref[pl.ds(half * L + r0, nr), :] += p

    wait_all(g0)
    k_pass(0, 0, 0, _L0, False)
    wait_all(g1)
    k_pass(0, 0, _L0, _L1 - _L0, False)
    wait_all(g2)
    k_pass(0, 0, _L1, L - _L1, True)
    k_pass(0, 1, 0, L, True)
    wait_all(g3)
    k_pass(1, 0, 0, L, True)
    dwf = dw_in[...].astype(f32) * 0.25
    for k in range(K):
        for c in range(NC):
            dwb_ref[c, k] = jnp.broadcast_to(dwf[k:k + 1, c * 128:(c + 1) * 128], (8, 128))
    k_pass(1, 1, 0, L, True)
    wait_all(g4)
    x23 = xb[pl.ds(0, L), 256:512]
    for c in range(NC):
        wa = w1b[256:512, c * 128:(c + 1) * 128]
        wg = w1b[256:512, D + c * 128:D + (c + 1) * 128]
        w1u[c, 128:256, :] = pltpu.bitcast(wa, u32)
        w1u[NC + c, 128:256, :] = pltpu.bitcast(wg, u32)
        q = jnp.dot(x23, jnp.concatenate([wa, wg], axis=1), preferred_element_type=f32)
        a = acc_ref[pl.ds(0, L), c * 128:(c + 1) * 128] + q[:, :128]
        g = acc_ref[pl.ds(L, L), c * 128:(c + 1) * 128] + q[:, 128:]
        glu_store(c, a, g, 0, L)
    w2_cp.wait()

    bt, boff = divmod(T, TT)
    RA = L - 16
    RB = TT - RA

    def body(i, carry):
        base = pl.multiple_of(i * TT, 32)
        x_cp(L + base, TT, S_X + i).wait()
        at_b = i == bt
        direct = {boff - 8: dict(hi_pred=at_b), boff: dict(lo_pred=at_b)}
        x = xb[pl.ds(base + L, TT), :]
        a = a_pass(0, x)
        out_pass(0, base, 0, RA, direct, 0, pack_w=True)
        for c in range(NC):
            g_pass(c, x, a, base + L, TT)
            if c + 1 < NC:
                a = a_pass(c + 1, x)
                out_pass(c + 1, base, 0, RA, direct, 0, pack_w=True)
            out_pass(c, base, RA, RB, direct, RA)
        return carry

    lax.fori_loop(0, _NT, body, 0)

    r0 = _NT * TT
    for nr in _EPI:
        for c in range(NC):
            out_pass(c, 0, r0, nr, {G - 8: {}}, r0 - _NT * TT)
        r0 += nr

    pltpu.make_async_copy(ob, o_hbm, sems.at[S_OUT]).wait()


@jax.jit
def pallas_standalone__conformer_conv_module__speech_kernel(
    x: jax.Array,
    w_pw1: jax.Array,
    dw: jax.Array,
    w_pw2: jax.Array,
):
    B, T, D = x.shape
    K = dw.shape[0]
    G = B * T
    NC = D // 128
    TT = (G - _LAG) // _NT
    boff = T % TT
    assert B == 2 and D == 512 and K == 15
    assert _LAG + _NT * TT == G and TT % 32 == 0 and sum(_EPI) == _LAG and _LAG - 16 < TT
    assert T < _NT * TT and boff % 8 == 0 and 8 <= boff <= TT - 8

    kernel = functools.partial(_kernel, G=G, T=T, K=K, D=D, TT=TT)
    out = pl.pallas_call(
        kernel,
        in_specs=[pl.BlockSpec(memory_space=pl.ANY)] * 4,
        out_specs=pl.BlockSpec(memory_space=pl.ANY),
        out_shape=jax.ShapeDtypeStruct((G, D), x.dtype),
        scratch_shapes=[
            pltpu.VMEM((G, D), jnp.bfloat16),
            pltpu.VMEM((D, 2 * D), jnp.bfloat16),
            pltpu.VMEM((D, D), jnp.bfloat16),
            pltpu.VMEM((K, D), jnp.bfloat16),
            pltpu.VMEM((G, D), jnp.bfloat16),
            pltpu.VMEM((NC, G + 2 * _H0, 128), jnp.float32),
            pltpu.VMEM((_PBASE[-1], G + 2 * _H0, 128), jnp.float32),
            pltpu.VMEM((NC, K, 8, 128), jnp.float32),
            pltpu.VMEM((max(TT, 2 * _LAG), D), jnp.float32),
            pltpu.VMEM((2 * NC, D // 2, 128), jnp.uint32),
            pltpu.VMEM((NC, 64, D), jnp.uint32),
            pltpu.SemaphoreType.DMA((7 + _NT,)),
        ],
        compiler_params=pltpu.CompilerParams(
            vmem_limit_bytes=108 * 1024 * 1024,
            disable_bounds_checks=True,
            disable_semaphore_checks=True,
        ),
    )(x.reshape(G, D), w_pw1, dw, w_pw2)
    return out.reshape(B, T, D)
```

```python
import functools

import jax
import jax.numpy as jnp
from jax import lax
import jax.experimental.pallas as pl
import jax.experimental.pallas.tpu as pltpu

_PRO = 1600
_LAG = 704
_L0 = 128
_L1 = 752
_NT = 4
_OCH = 3
_OFFS = ((1, 2, 3), (1, 2, 3, 4), (1, 2, 3, 4), (1, 2, 3))
_PBASE = (0, 3, 7, 11, 14)
_EPI = (320, 176, 96, 48, 32, 32)
_H0 = 32


def _tree_sum(terms):
    while len(terms) > 1:
        nxt = [terms[j] + terms[j + 1] for j in range(0, len(terms) - 1, 2)]
        if len(terms) % 2:
            nxt.append(terms[-1])
        terms = nxt
    return terms[0]


def _kernel(x_hbm, w1_hbm, dw_hbm, w2_hbm, o_hbm,
            xb, w1b, w2b, dw_in, ob, h_ref, p_ref, dwb_ref, acc_ref, w1u, w2u, sems,
            *, G, T, K, D, TT):
    L, LAG, H0 = _PRO, _LAG, _H0
    O0 = L - LAG
    NC = D // 128
    P = K // 2
    f32, bf16, u32 = jnp.float32, jnp.bfloat16, jnp.uint32
    S_G0, S_G1, S_G2, S_G3, S_G4, S_OUT, S_X = range(7)

    def w1_cp(r0, nr, c0, nc, s):
        sl = (pl.ds(r0, nr), pl.ds(c0, nc))
        return pltpu.make_async_copy(w1_hbm.at[sl], w1b.at[sl], sems.at[s])

    def xcol_cp(r0, nr, c0, nc, s):
        sl = (pl.ds(r0, nr), pl.ds(c0, nc))
        return pltpu.make_async_copy(x_hbm.at[sl], xb.at[sl], sems.at[s])

    def x_cp(r0, nr, s):
        return pltpu.make_async_copy(x_hbm.at[pl.ds(r0, nr)], xb.at[pl.ds(r0, nr)], sems.at[s])

    def o_cp(r0, nr):
        return pltpu.make_async_copy(ob.at[pl.ds(r0, nr)], o_hbm.at[pl.ds(r0, nr)], sems.at[S_OUT])

    def wait_all(cps):
        for cp in cps:
            cp.wait()

    g0 = [w1_cp(0, 128, 0, D, S_G0), xcol_cp(0, _L0, 0, 128, S_G0)]
    g1 = [xcol_cp(_L0, _L1 - _L0, 0, 128, S_G1)]
    g2 = [xcol_cp(_L1, L - _L1, 0, 128, S_G2), w1_cp(0, 128, D, D, S_G2)]
    g3 = [pltpu.make_async_copy(dw_hbm, dw_in, sems.at[S_G3]),
          xcol_cp(0, L, 128, 128, S_G3), w1_cp(128, 128, 0, 2 * D, S_G3)]
    g4 = [xcol_cp(0, L, 256, 256, S_G4), w1_cp(256, 256, 0, 2 * D, S_G4),
          pltpu.make_async_copy(w2_hbm, w2b, sems.at[S_G4])]

    for cp in g0 + g1 + g2 + g3 + g4:
        cp.start()
    for t in range(_NT):
        x_cp(L + t * TT, TT, S_X + t).start()

    zero = jnp.zeros((8, 128), f32)
    for c in range(NC):
        h_ref[c, pl.ds(H0 - 8, 8), :] = zero
        h_ref[c, pl.ds(H0 + G, 8), :] = zero

    def glu_store(c, a, g, r0, nr):
        h = a + a * jnp.tanh(0.5 * g)
        h_ref[c, pl.ds(r0 + H0, nr), :] = h
        hprev = h_ref[c, pl.ds(r0 + (H0 - 8), 8), :]
        h3 = h.reshape(nr // 8, 8, 128)
        hm = jnp.concatenate([hprev[None], h3[:-1]], axis=0)
        for oi, o in enumerate(_OFFS[c]):
            pv = h3 * dwb_ref[c, P + o][None] + hm * dwb_ref[c, o - 1][None]
            p_ref[_PBASE[c] + oi, pl.ds(r0 + H0, nr), :] = pv.reshape(nr, 128)

    def a_pass(c, x):
        return jnp.dot(x, pltpu.bitcast(w1u[c], bf16), preferred_element_type=f32)

    def g_pass(c, x, a, r0, nr):
        g = jnp.dot(x, pltpu.bitcast(w1u[NC + c], bf16), preferred_element_type=f32)
        glu_store(c, a, g, r0, nr)

    rows = lax.broadcasted_iota(jnp.int32, (8, 128), 0)

    def conv_direct(c, r0, lo_pred=None, hi_pred=None):
        terms = []
        for k in range(K):
            hv = h_ref[c, pl.ds(r0 + (H0 + k - P), 8), :]
            if lo_pred is not None and k < P:
                hv = jnp.where(rows >= jnp.where(lo_pred, P - k, 0), hv, 0.0)
            if hi_pred is not None and k > P:
                hv = jnp.where(rows < jnp.where(hi_pred, 8 - (k - P), 8), hv, 0.0)
            terms.append(hv * dwb_ref[c, k])
        return _tree_sum(terms)[None]

    def conv_paired(c, r0, nr):
        terms = []
        for k in range(K):
            o = k - P
            if o in _OFFS[c] or (o + 8) in _OFFS[c]:
                continue
            hv = h_ref[c, pl.ds(r0 + (H0 + o), nr), :].reshape(nr // 8, 8, 128)
            terms.append(hv * dwb_ref[c, k][None])
        for oi, o in enumerate(_OFFS[c]):
            pv = p_ref[_PBASE[c] + oi, pl.ds(r0 + (H0 + o), nr), :]
            terms.append(pv.reshape(nr // 8, 8, 128))
        return _tree_sum(terms)

    def conv(c, base, s0, nr, direct):
        parts = []
        r = s0
        for sr in sorted(direct):
            if s0 <= sr < s0 + nr:
                if sr > r:
                    parts.append(conv_paired(c, base + r, sr - r))
                parts.append(conv_direct(c, base + sr, **direct[sr]))
                r = sr + 8
        if r < s0 + nr:
            parts.append(conv_paired(c, base + r, s0 + nr - r))
        y = jnp.concatenate(parts, axis=0) if len(parts) > 1 else parts[0]
        return y.reshape(nr, 128)

    def out_pass(c, base, s0, nr, direct, a0, pack_w=False, och=1):
        y = conv(c, base, s0, nr, direct)
        s = (y + y * jnp.tanh(y)).astype(bf16)
        if pack_w:
            w = w2b[c * 128:(c + 1) * 128, :]
            w2u[c] = pltpu.bitcast(w, u32)
        else:
            w = pltpu.bitcast(w2u[c], bf16)
        p = jnp.dot(s, w, preferred_element_type=f32)
        if c == 0:
            acc_ref[pl.ds(a0, nr), :] = p
        elif c < NC - 1:
            acc_ref[pl.ds(a0, nr), :] += p
        else:
            g16 = nr // 16
            q0 = 0
            for j in range(och):
                q = 16 * (g16 // och + (1 if j < g16 % och else 0))
                ob[pl.ds(base + (s0 + q0), q), :] = (
                    acc_ref[pl.ds(a0 + q0, q), :] + p[q0:q0 + q]).astype(ob.dtype)
                o_cp(base + (s0 + q0), q).start()
                q0 += q

    def k_pass(k, half, r0, nr, pack_w):
        w = w1b[k * 128:(k + 1) * 128, half * D:(half + 1) * D]
        if pack_w:
            wu = pltpu.bitcast(w, u32)
            for c in range(NC):
                w1u[half * NC + c, k * 64:(k + 1) * 64, :] = wu[:, c * 128:(c + 1) * 128]
        p = jnp.dot(xb[pl.ds(r0, nr), k * 128:(k + 1) * 128], w, preferred_element_type=f32)
        if k == 0:
            acc_ref[pl.ds(half * L + r0, nr), :] = p
        else:
            acc_ref[pl.ds(half * L + r0, nr), :] += p

    wait_all(g0)
    k_pass(0, 0, 0, _L0, False)
    wait_all(g1)
    k_pass(0, 0, _L0, _L1 - _L0, False)
    wait_all(g2)
    k_pass(0, 0, _L1, L - _L1, True)
    k_pass(0, 1, 0, L, True)
    wait_all(g3)
    k_pass(1, 0, 0, L, True)
    dwf = dw_in[...].astype(f32) * 0.25
    for k in range(K):
        for c in range(NC):
            dwb_ref[c, k] = jnp.broadcast_to(dwf[k:k + 1, c * 128:(c + 1) * 128], (8, 128))
    k_pass(1, 1, 0, L, True)
    wait_all(g4)
    x23 = xb[pl.ds(0, L), 256:512]
    for c in range(NC):
        wa = w1b[256:512, c * 128:(c + 1) * 128]
        wg = w1b[256:512, D + c * 128:D + (c + 1) * 128]
        w1u[c, 128:256, :] = pltpu.bitcast(wa, u32)
        w1u[NC + c, 128:256, :] = pltpu.bitcast(wg, u32)
        q = jnp.dot(x23, jnp.concatenate([wa, wg], axis=1), preferred_element_type=f32)
        a = acc_ref[pl.ds(0, L), c * 128:(c + 1) * 128] + q[:, :128]
        g = acc_ref[pl.ds(L, L), c * 128:(c + 1) * 128] + q[:, 128:]
        glu_store(c, a, g, 0, L)
    for c in range(NC):
        out_pass(c, 0, 0, O0, {}, 2 * L, pack_w=True)

    bt, boff = divmod(T - O0, TT)
    boff += O0
    RA = LAG - 16
    RB = TT - RA

    def body(i, carry):
        base = pl.multiple_of(i * TT, 32)
        x_cp(L + base, TT, S_X + i).wait()
        at_b = i == bt
        direct = {boff - 8: dict(hi_pred=at_b), boff: dict(lo_pred=at_b)}
        x = xb[pl.ds(base + L, TT), :]
        a = a_pass(0, x)
        out_pass(0, base, O0, RA, direct, 0)
        for c in range(NC):
            g_pass(c, x, a, base + L, TT)
            if c + 1 < NC:
                a = a_pass(c + 1, x)
                out_pass(c + 1, base, O0, RA, direct, 0)
            out_pass(c, base, O0 + RA, RB, direct, RA, och=_OCH)
        return carry

    lax.fori_loop(0, _NT, body, 0)

    r0 = G - LAG
    for nr in _EPI:
        for c in range(NC):
            out_pass(c, 0, r0, nr, {G - 8: {}}, r0 - (G - LAG))
        r0 += nr

    pltpu.make_async_copy(ob, o_hbm, sems.at[S_OUT]).wait()


@jax.jit
def pallas_standalone__conformer_conv_module__speech_kernel(
    x: jax.Array,
    w_pw1: jax.Array,
    dw: jax.Array,
    w_pw2: jax.Array,
):
    B, T, D = x.shape
    K = dw.shape[0]
    G = B * T
    NC = D // 128
    TT = (G - _PRO) // _NT
    boff = (T - (_PRO - _LAG)) % TT
    assert B == 2 and D == 512 and K == 15
    assert _PRO + _NT * TT == G and TT % 32 == 0 and sum(_EPI) == _LAG and _LAG - 16 < TT
    assert _PRO < T < G - _LAG and boff % 8 == 0 and 8 <= boff <= TT - 8

    kernel = functools.partial(_kernel, G=G, T=T, K=K, D=D, TT=TT)
    out = pl.pallas_call(
        kernel,
        in_specs=[pl.BlockSpec(memory_space=pl.ANY)] * 4,
        out_specs=pl.BlockSpec(memory_space=pl.ANY),
        out_shape=jax.ShapeDtypeStruct((G, D), x.dtype),
        scratch_shapes=[
            pltpu.VMEM((G, D), jnp.bfloat16),
            pltpu.VMEM((D, 2 * D), jnp.bfloat16),
            pltpu.VMEM((D, D), jnp.bfloat16),
            pltpu.VMEM((K, D), jnp.bfloat16),
            pltpu.VMEM((G, D), jnp.bfloat16),
            pltpu.VMEM((NC, G + 2 * _H0, 128), jnp.float32),
            pltpu.VMEM((_PBASE[-1], G + 2 * _H0, 128), jnp.float32),
            pltpu.VMEM((NC, K, 8, 128), jnp.float32),
            pltpu.VMEM((3 * _PRO - _LAG, D), jnp.float32),
            pltpu.VMEM((2 * NC, D // 2, 128), jnp.uint32),
            pltpu.VMEM((NC, 64, D), jnp.uint32),
            pltpu.SemaphoreType.DMA((6 + _NT,)),
        ],
        compiler_params=pltpu.CompilerParams(
            vmem_limit_bytes=112 * 1024 * 1024,
            disable_bounds_checks=True,
            disable_semaphore_checks=True,
        ),
    )(x.reshape(G, D), w_pw1, dw, w_pw2)
    return out.reshape(B, T, D)
```
